```python
import os as _os
_os.environ.setdefault("JAX_PLATFORMS", "cpu")
import jax
import jax.numpy as jnp

def _softmax(x, axis=-1):
    return jax.nn.softmax(x, axis=axis)
def _gelu(x):
    return jax.nn.gelu(x, approximate=True)
def _silu(x):
    return jax.nn.silu(x)
def _sigmoid(x):
    return jax.nn.sigmoid(x)
def _layernorm(x, axis=-1, eps=1e-5):
    m = jnp.mean(x, axis=axis, keepdims=True)
    v = jnp.var(x, axis=axis, keepdims=True)
    return (x - m) / jnp.sqrt(v + eps)
def _scatter_add(tgt, idx, src, axis=0):
    return tgt.at[idx].add(src)
def _segment_sum(src, seg, n):
    return jax.ops.segment_sum(src, seg, n)
class _Rng:
    def __init__(self, key):
        self._k = key
    def _next(self):
        self._k, sub = jax.random.split(self._k)
        return sub
    def normal(self, shape):
        return jax.random.normal(self._next(), shape, dtype=jnp.bfloat16)
    def randint(self, lo, hi, shape):
        return jax.random.randint(self._next(), shape, lo, hi, dtype=jnp.int32)
    def uniform(self, shape, lo=0.0, hi=1.0):
        return jax.random.uniform(self._next(), shape, jnp.bfloat16, lo, hi)
    def permutation(self, n):
        return jax.random.permutation(self._next(), n)


kernel_name = 'sequential_preLN__sliding_block__mixer_channel_mlp__prompt'

def setup_inputs():
    _rng = _Rng(jax.random.key(int.from_bytes(__import__("os").urandom(4), "little")))
    _w = (lambda a: (lambda t: t.astype(jnp.bfloat16) if jnp.issubdtype(t.dtype, jnp.floating) else t)(jnp.asarray(a)))
    def _A_setup():
        B, S, D = 1, 2048, 1024
        return {
            "x": _w((lambda *s: _rng.normal(s) * 0.05)(B, S, D)),
            "wqkv": _w((lambda *s: _rng.normal(s) * 0.05)(D, 3 * D)),
            "wo": _w((lambda *s: _rng.normal(s) * 0.05)(D, D)),
        }
    _A_in = _A_setup()

    def _B_setup():
        B, S, D, F = 1, 2048, 1024, 3584
        return {
            "x": _w((lambda *s: _rng.normal(s) * 0.05)(B, S, D)),
            "w1": _w((lambda *s: _rng.normal(s) * 0.8)(D, F) * (D ** -0.5)),
            "b1": _w((lambda *s: _rng.normal(s) * 0.8)(F)),
            "w2": _w((lambda *s: _rng.normal(s) * 0.8)(F, D) * (F ** -0.5)),
            "b2": _w((lambda *s: _rng.normal(s) * 0.05)(D)),
        }
    _B_in = _B_setup()

    return {
        "A_x": _A_in["x"],
        "A_wqkv": _A_in["wqkv"],
        "A_wo": _A_in["wo"],
        "B_x": _B_in["x"],
        "B_w1": _B_in["w1"],
        "B_b1": _B_in["b1"],
        "B_w2": _B_in["w2"],
        "B_b2": _B_in["b2"],
    }

def reference(A_x, A_wqkv, A_wo, B_x, B_w1, B_b1, B_w2, B_b2):
    def _A_ref(x, wqkv, wo):
        B, S, D = x.shape
        H = 32; Dh = D // H; W = 256
        qkv = (lambda x, *d: x.transpose(*d))((x @ wqkv).reshape(B, S, 3, H, Dh), 2, 0, 3, 1, 4)
        q, k, v = qkv[0], qkv[1], qkv[2]
        scores = jnp.einsum("bhqd,bhkd->bhqk", q, k) * (Dh ** -0.5)
        idx = jnp.arange(S)
        mask = (idx[:, None] - idx[None, :] >= 0) & (idx[:, None] - idx[None, :] < W)
        scores = jnp.where(mask[None, None], scores, -1e9)
        p = _softmax(scores, axis=-1)
        o = jnp.einsum("bhqk,bhkd->bhqd", p, v)
        return (lambda x, *d: x.transpose(*d))(o, 0, 2, 1, 3).reshape(B, S, D) @ wo

    def _B_ref(x, w1, b1, w2, b2):
        y = _layernorm(x, axis=-1)
        h = _gelu(jnp.einsum("bsd,df->bsf", y, w1) + b1)
        return jnp.einsum("bsf,fd->bsd", h, w2) + b2

    x = A_x
    h = x + _A_ref(_layernorm(x, axis=-1), A_wqkv, A_wo)
    h2 = h + _B_ref(_layernorm(h, axis=-1), B_w1, B_b1, B_w2, B_b2)
    return h2
```

```python
import functools
import math

import jax
import jax.numpy as jnp
from jax import lax
from jax.experimental import pallas as pl
from jax.experimental.pallas import tpu as pltpu

H = 32
W = 256
EPS = 1e-5
T = 256
LG = 128
NEG = -1e30

f32 = jnp.float32
bf16 = jnp.bfloat16

OPT = dict(chain=3, gate1=2, anchor=1, flags={}, bc=1, ln2rows=32, ln1rows=32, lngate=0, lnlag=4, actspan=30, lt0=0, lt1=24, selfchain=0, tick0=0, tick1=0, actfrom=0, earlypad=3, ln1lag=2, ln1gate=2, defer=1, early=9, z1=0, reload=((0,),(1,4),(2,),(3,),(5,),(6,)), opaque=0, smem=1, mmem=1, unit=16, pmem=0, order='s0 k012 q0:12 v0 s1 k3456 q1:12 v1 f', order0='s0 k012 q0:12 v0 s1 k3456 q1:12 w v1 f', order7='s0 k012 q0:12 v0 k3456 v1 f q1', prep=1, only=None)


GELU_A = math.sqrt(2.0 / math.pi)
GELU_S = (GELU_A * 0.044715) ** (1.0 / 3.0)


def _layernorm(v, twice, gate=None, scale=1.0):
    m = jnp.mean(v, axis=-1, keepdims=True)
    if gate is not None:
        m = gate(m)
    c = v - m
    var = jnp.mean(c * c, axis=-1, keepdims=True)
    rs = lax.rsqrt(var + EPS)
    if twice:
        m = jnp.mean(c, axis=-1, keepdims=True)
        c = c - m
        var = jnp.mean(c * c, axis=-1, keepdims=True)
        rs = rs * lax.rsqrt(rs * rs * var + EPS)
    if scale != 1.0:
        rs = rs * scale
    return c * rs, (m, var, rs)


def _layernorm_chunks(chunks, twice, always, lag, which, scale=1.0, ticks=None):
    out, stats = [], []
    for c in chunks:
        gate = (lambda m: jnp.where(always, m, stats[-lag][which])) if lag and len(stats) >= lag else None
        if ticks:
            gate = lambda m: jnp.where(always, m, ticks[len(out) * len(ticks) // len(chunks)][:, 0:1])
        y, st = _layernorm(c, twice, gate, scale)
        out.append(y)
        stats.append(st)
    return out


def _gelu_scaled(u, k):
    return u + u * jnp.tanh(u * (k + u * u))


def _dot(a, b):
    return jnp.dot(a, b, preferred_element_type=f32)


def _dot_nt(a, b):
    return lax.dot_general(a, b, (((1,), (1,)), ((), ())), preferred_element_type=f32)


def _ld(ref, *idx):
    if not OPT["bc"]:
        return ref[idx]
    return pltpu.bitcast(ref.bitcast(jnp.uint32)[idx], bf16)


def _rows(start, size):
    if not OPT["bc"]:
        return pl.ds(start, size)
    if isinstance(start, int):
        return pl.ds(start // 2, size // 2)
    return pl.ds(pl.multiple_of(start // 2, 8), size // 2)


def _s_lhs(a11, a12, a21, a22):
    return [a11 + a22, a21 + a22, a11, a22, a11 + a12, a21 - a11, a12 - a22]


def _s_rhs(b11, b12, b21, b22):
    return [b11 + b22, b11, b12 - b22, b21 - b11, b22, b11 + b12, b21 + b22]


def _s_out(m):
    return [m[0] + m[3] - m[4] + m[6], m[2] + m[4], m[1] + m[3], m[0] - m[1] + m[2] + m[5]]


def _two_level(rule, blk):
    outer = [rule(*[blk[2 * I + i][2 * J + j] for I in range(2) for J in range(2)])
             for i in range(2) for j in range(2)]
    return [v for k in range(7) for v in rule(*[outer[q][k] for q in range(4)])]


def _xor_shuffle(blocks, g0, g1):
    def sel(m, a, b):
        if a is None and b is None:
            return None
        if a is None:
            a = jnp.zeros_like(b)
        if b is None:
            b = jnp.zeros_like(a)
        return jnp.where(m, a, b)
    a = [sel(g0, blocks[j ^ 1], blocks[j]) for j in range(4)]
    return [sel(g1, a[j ^ 2], a[j]) for j in range(4)]


def _tree_sum(vs):
    while len(vs) > 1:
        vs = [vs[i] + vs[i + 1] if i + 1 < len(vs) else vs[i] for i in range(0, len(vs), 2)]
    return vs[0]


class _Attn:
    def __init__(self, flag, sbuf, pbuf):
        lane = lax.broadcasted_iota(jnp.int32, (32, LG), 1)
        self.g0 = (lane & 32) != 0
        self.g1 = (lane & 64) != 0
        self.hmask = [(lane >> 5) == h for h in range(4)]
        self.tri = lax.broadcasted_iota(jnp.int32, (32, LG), 0) > (lane & 31)
        lane1 = lax.broadcasted_iota(jnp.int32, (1, LG), 1)
        self.g0r = (lane1 & 32) != 0
        self.g1r = (lane1 & 64) != 0
        self.always = flag > 0
        self.zero = flag - 1
        self.sbuf = sbuf
        self.pbuf = pbuf

    def scores(self, slot, q, kwin, first=None, nprev=0):
        skip = (W + 128 - kwin.shape[0]) // 32
        m = []
        sv = {}
        for t in range(4):
            qt = q[32 * t:32 * t + 32].astype(f32)
            rhs = jnp.concatenate(
                [jnp.where(self.hmask[g ^ t], qt, 0.0) for g in range(4)], axis=0).astype(bf16)
            c0 = max(skip - t, 0)
            s = _dot_nt(kwin[32 * (t + c0 - skip):32 * (t + 9 - skip)], rhs)
            s = {c: s[32 * (c - c0):32 * (c - c0 + 1)] for c in range(c0, 9)}
            if c0 > 0:
                s[0] = jnp.where(self.tri, NEG, s[8])
            elif first is None:
                s[0] = jnp.where(self.tri, s[0], s[8])
            else:
                s[0] = jnp.where(self.tri, jnp.where(first, NEG, s[0]), s[8])
            del s[8]
            npv = 0 if first is None else nprev - t
            mx = functools.reduce(jnp.maximum, [s[c] for c in range(max(1, npv, c0), 8)] + [s[0]])
            if npv > 1:
                mx = jnp.maximum(mx, jnp.where(
                    first, NEG, functools.reduce(jnp.maximum, [s[c] for c in range(1, npv)])))
            m.append(jnp.broadcast_to(jnp.max(mx, axis=0, keepdims=True), (8, LG)))
            for c, v in s.items():
                if OPT["smem"]:
                    self.sbuf[slot][t, c] = v
                sv[t, c] = v
        return functools.partial(self.probs, slot, skip, m, sv, first, nprev)

    def probs(self, slot, skip, m, sv, first, nprev, ticks):
        U = OPT["unit"]
        links = 0
        l = [None] * 4
        tail = {}
        rows = []
        gate, pending, touched = None, 0, set()
        for r in range(12):
            for lo in range(0, 32, U):
                blk = [None] * 4
                for t in range(4):
                    c = r - t
                    if c == 8:
                        blk[t] = tail[t, lo]
                    if (t, c) not in sv:
                        continue
                    mr = m[t]
                    if gate is not None:
                        mr = jnp.where(self.always, mr, gate)
                    if c > 0 and first is not None and r < nprev:
                        mr = jnp.where(first, -NEG, mr)
                    sc = self.sbuf[slot][t + self.zero, c, lo:lo + U] if OPT["smem"] else sv[t, c][lo:lo + U]
                    p = jnp.exp2(sc - jnp.concatenate([mr] * (U // 8), axis=0))
                    f = _tree_sum([p[i:i + 8] for i in range(0, U, 8)])
                    l[t] = f if l[t] is None else l[t] + f
                    pending += 1
                    touched.add(t)
                    if c == 0:
                        tail[t, lo] = jnp.where(self.tri[lo:lo + U], 0.0, p)
                        p = None if t < skip else jnp.where(self.tri[lo:lo + U], p, 0.0)
                    blk[t] = p
                if any(v is not None for v in blk):
                    out = _xor_shuffle(blk, self.g0[:U], self.g1[:U])
                    if OPT["pmem"]:
                        for h in range(4):
                            self.pbuf[slot][h, 32 * r + lo:32 * r + lo + U] = out[h].astype(bf16)
                    rows.append(out)
                if OPT["chain"] and pending >= OPT["chain"]:
                    ts = sorted(touched)
                    if OPT["gate1"]:
                        ts = ts[-OPT["gate1"]:]
                    z = [l[t] for t in ts] if OPT["selfchain"] or not ticks else []
                    if ticks:
                        z.append(ticks[min(len(ticks) - 1, links * len(ticks) * OPT["chain"] // 64)])
                    links += 1
                    gate, pending, touched = _tree_sum(z), 0, set()
        inv = _xor_shuffle([1.0 / jnp.sum(v, axis=0, keepdims=True) for v in l], self.g0r, self.g1r)
        if OPT["pmem"]:
            return lambda h: _ld(self.pbuf[slot], h + self.zero, _rows(32 * skip, 384 - 32 * skip)), inv
        return lambda h: jnp.concatenate([row[h] for row in rows], axis=0).astype(bf16), inv

    def values(self, pr, vt):
        pt, inv = pr
        ot = [_dot(jnp.concatenate([v[32 * h:32 * h + 32] for v in vt], axis=1), pt(h)) * inv[h]
              for h in range(4)]
        o = jnp.concatenate(ot, axis=0).T
        o = _xor_shuffle([o[32 * j:32 * j + 32] for j in range(4)], self.g0, self.g1)
        return jnp.concatenate(o, axis=0)


def _kernel(x_hbm, wqkv_hbm, wo_hbm, w1_hbm, b1_ref, w2_hbm, b2_ref, out_hbm,
            xv, wkv, wkvs, wo, w1, w2, big, qb_, kb, vb, ob, a1, a2, c11, bias, obuf,
            sb0, sb1, pb0, pb1, mbuf, flag, xsem, wsem, osem, *, S, D, F):
    NB = S // T
    NG = D // LG
    FC = 4 * LG
    NF = F // FC
    HT = T // 2
    QT = T // 4
    qscale = (D // H) ** -0.5 * math.log2(math.e)
    def tile(k, j):
        return 16 * (98 * j + k)

    def ytile(b, i, c):
        return 16 * 98 * NF + 8 * (4 * (9 * b + i) + c)

    def otile(i, c):
        return ytile(NB, 0, 0) + 32 * (4 * i + c)

    def ld_tiles(ref, at, n):
        v = ref.bitcast(jnp.uint32)[pl.ds(at, n)]
        return pltpu.bitcast(v.reshape(8 * n, LG), bf16)

    ld_big = functools.partial(ld_tiles, big)

    def x_copy(i):
        return pltpu.make_async_copy(x_hbm.at[0, pl.ds(i * T, T)], xv.at[i], xsem.at[i])

    def o_copy(i):
        return pltpu.make_async_copy(obuf.at[i + 1], out_hbm.at[0, pl.ds(i * T, T)], osem.at[i])

    def qkv_copies(g):
        return [pltpu.make_async_copy(wqkv_hbm.at[:, pl.ds((p + 1) % 3 * D + g * LG, LG)],
                                      wkv.at[g, p], wsem.at[p // 2, g]) for p in range(3)]

    def mlp_copies(j):
        return [pltpu.make_async_copy(w1_hbm.at[:, pl.ds(j * FC, FC)], w1.at[j], wsem.at[2, j]),
                pltpu.make_async_copy(w2_hbm.at[pl.ds(j * FC, FC), :], w2.at[j], wsem.at[2, j])]

    wo_copy = pltpu.make_async_copy(wo_hbm, wo, wsem.at[2, NF])

    x_copy(0).start()
    for cp in qkv_copies(0):
        cp.start()
    for i in range(1, NB):
        x_copy(i).start()
    for cp in qkv_copies(1) + mlp_copies(0):
        cp.start()

    kb[0:W] = jnp.zeros((W, LG), bf16)
    vb[0:W // LG] = jnp.zeros((W // LG, LG, LG), bf16)
    a2[42:49] = jnp.zeros((7,) + a2.shape[1:], bf16)
    c11[...] = jnp.zeros_like(c11)
    flag[0] = 1
    for i in range(1, 8):
        flag[i] = 0
    bias[:, 0:F] = jnp.broadcast_to(b1_ref[...].astype(f32).reshape(1, F) * GELU_S, (8, F))
    bias[:, F:F + D] = jnp.broadcast_to(b2_ref[...].astype(f32).reshape(1, D), (8, D))

    def ln1(b, lag):
        ys = _layernorm_chunks([xv[b, r * HT + k:r * HT + k + 16].astype(f32)
                                for k in range(0, HT, 16) for r in range(2)],
                               False, flag[0] > 0, lag, OPT["ln1gate"])
        for k in range(HT // 16):
            for c in range(4):
                quad = [ys[2 * k + r][:, p * (D // 2) + c * LG:p * (D // 2) + (c + 1) * LG]
                        for r in range(2) for p in range(2)]
                for i, v in enumerate(_s_lhs(*quad) + [quad[1], quad[2]]):
                    big[ytile(b, 0, 0) + (ytile(0, i, c) - ytile(0, 0, 0) + k)] = v.astype(bf16)

    def y_op(b, i, between=None):
        if between is None:
            return jnp.concatenate(
                [ld_big(ytile(b, i, c), 8) for c in range(4)], axis=1)
        parts = []
        zero = flag[1]
        for r in range(0, HT, 16):
            between()
            parts.append(jnp.concatenate(
                [ld_big(zero + (ytile(b, i, c) + r // 16), 1) for c in range(4)],
                axis=1))
        return jnp.concatenate(parts, axis=0)

    def y_rows(b, r, between):
        return jnp.concatenate([y_op(b, (2, 8)[r], between), y_op(b, (7, 3)[r], between)], axis=1)

    def proj_q(g, b, r, between=None):
        wq = _ld(wkv, g, 2)
        q = _dot(y_rows(b, r, between), wq) * qscale
        qb_[pl.ds(b * T + r * HT, HT)] = q.astype(bf16)
        return q

    def prep_kv(g):
        for k in range(0, D // 2, 16):
            ops = _s_rhs(*[wkv[g, p, r * (D // 2) + k:r * (D // 2) + k + 16].astype(f32)
                           for r in range(2) for p in range(2)])
            for i, n in enumerate((0, 2, 3, 5, 6)):
                wkvs[i, k:k + 16] = ops[n].astype(bf16)

    def kv_product(g, b, i, between=None):
        if i == 1:
            rhs = _ld(wkv, g, 0, _rows(0, D // 2))
        elif i == 4:
            rhs = _ld(wkv, g, 1, _rows(D // 2, D // 2))
        else:
            rhs = _ld(wkvs, (0, 2, 3, 5, 6).index(i))
        m = _dot(y_op(b, i, between), rhs)
        if OPT["mmem"] and i < 6:
            mbuf[i] = m
        return m

    def put_kv(b, m, parts="kv"):
        if OPT["mmem"]:
            m = [mbuf[i + flag[0] - 1] for i in range(6)] + [m[6]]
        c = _s_out(m)
        for r in range(2):
            if "k" in parts:
                kb[pl.ds(W + b * T + r * HT, HT)] = c[2 * r].astype(bf16)
            if "v" in parts:
                vb[2 + 2 * b + r] = c[2 * r + 1].T.astype(bf16)

    def prep_mlp(j, pos, which, z, ks):
        n, rr = divmod(pos, 8)

        def load(r, c):
            if which == 0:
                return w1[j + z, pl.ds(256 * r + 16 * pos, 16), c * LG:(c + 1) * LG].astype(f32)
            return w2[j + z, pl.ds(LG * r + 16 * rr, 16), 256 * c + LG * n:256 * c + LG * (n + 1)].astype(f32)

        ops = _two_level(_s_rhs, [[load(r, c) for c in range(4)] for r in range(4)])
        for k in ks:
            for kk in range(7 * k, 7 * k + 7):
                big[tile(0, j) + (tile(49 * which + kk, 0) + pos)] = ops[kk].astype(bf16)

    def spread(steps, n, slots):
        count = [0]

        def between():
            count[0] += 1
            for _ in range(n * count[0] // slots - n * (count[0] - 1) // slots):
                steps.pop(0)()
        return between if n else None

    x_copy(0).wait()
    ln1(0, 0)
    for cp in qkv_copies(0)[:2]:
        cp.wait()
    prep_kv(0)
    qkv_copies(0)[2].wait()

    def phase0(b, carry):
        x_copy(b + 1).wait()
        put_kv(b, [kv_product(0, b, i) for i in range(7)])
        for r in range(2):
            proj_q(0, b, r)
        ln1(b + 1, OPT["ln1lag"])
        return carry

    if OPT['only'] in (None, 0):
        lax.fori_loop(0, NB - 1, phase0, None)
    for j in range(1, NF):
        for cp in qkv_copies(j + 1) + mlp_copies(j):
            cp.start()
    wo_copy.start()

    def phase1(g, carry):
        for cp in qkv_copies(g + 1) + mlp_copies(g):
            cp.wait()
        at = _Attn(flag[0], (sb0, sb1), (pb0, pb1))

        def scores(u):
            lo = max(u * HT, W)
            return at.scores(u % 2, qb_[u * HT:(u + 1) * HT], _ld(kb, _rows(lo, (u + 1) * HT + W - lo)))

        def values(u, pr):
            o = at.values(pr(ticks.pop(u)[OPT['tick0']:OPT['tick1']]), [_ld(vb, j) for j in range(max(u, 2), u + 3)])
            ob[g, u * HT:(u + 1) * HT] = o.astype(bf16)
            return o

        steps = [functools.partial(prep_mlp, g, pos, which, 0, ks)
                 for pos in range(16) for which in range(2) for ks in OPT["reload"]]
        ticks = {0: []}
        issued = set()
        orders = [OPT.get("order%d" % b, OPT["order"]).split() for b in range(NB)]
        total = sum(int(op.partition(":")[2] or 0) for o in orders for op in o)
        nsteps, used = len(steps), 0
        pr = {0: scores(0)}
        for b in range(NB):
            gp, bp = (g, NB - 1) if b == 0 else (g + 1, b - 1)
            m = []
            for op in orders[b]:
                op, _, n = op.partition(":")
                n, used = nsteps * (used + int(n or 0)) // total - nsteps * used // total, used + int(n or 0)
                if op[0] == "s":
                    u = 2 * b + 1 + int(op[1])
                    if u < 2 * NB and u not in issued:
                        issued.add(u)
                        pr[u] = scores(u)
                        ticks[u] = []
                elif op[0] == "v":
                    u = 2 * b + int(op[1])
                    values(u, pr.pop(u))
                elif op[0] == "k":
                    between = spread(steps, n * OPT['prep'], 8 * len(op[1:]))
                    for i in op[1:]:
                        m.append(kv_product(gp, bp, int(i), between))
                        for t in ticks.values():
                            t += [m[-1][r:r + 8] for r in range(0, HT, 32)]
                elif op[0] == "q":
                    q = proj_q(gp, bp, int(op[1]), spread(steps, n * OPT['prep'], 16))
                    for t in ticks.values():
                        t += [q[r:r + 8] for r in range(0, HT, 32)]
                elif op[0] == "f":
                    assert b == 0 or not any(u <= 2 * bp + 3 for u in pr)
                    put_kv(bp, m)
                elif op[0] == "w":
                    prep_kv(g + 1)
        assert not steps or not OPT['prep'], len(steps)
        return carry

    if OPT['only'] in (None, 1):
        lax.fori_loop(0, NG - 1, phase1, None)
    if OPT['only'] in (0, 1):
        pltpu.sync_copy(ob.at[0], out_hbm.at[0, :, pl.ds(0, 128)])
        pltpu.sync_copy(big.at[flag[1]], out_hbm.at[0, pl.ds(0, 16), pl.ds(0, 128)])
        pltpu.sync_copy(qb_, out_hbm.at[0, :, pl.ds(0, 128)])
        pltpu.sync_copy(kb.at[pl.ds(0, S)], out_hbm.at[0, :, pl.ds(0, 128)])
        pltpu.sync_copy(vb.at[0], out_hbm.at[0, pl.ds(0, 128), pl.ds(0, 128)])
        return

    def prep_wo(c, k):
        ops = _s_rhs(*[wo[r * (D // 2) + 16 * k:r * (D // 2) + 16 * k + 16,
                          p * (D // 2) + c * LG:p * (D // 2) + (c + 1) * LG].astype(f32)
                       for r in range(2) for p in range(2)])
        for i, n in enumerate((0, 2, 3, 5, 6)):
            big[otile(i, c) + k] = ops[n].astype(bf16)

    wo_copy.wait()
    steps = [functools.partial(prep_wo, c, k) for c in range(4) for k in range(D // 32)]
    between = spread(steps, len(steps), 88)
    put_kv(NB - 1, [kv_product(NG - 1, NB - 1, i, between) for i in range(7)])
    for r in range(2):
        proj_q(NG - 1, NB - 1, r, between)

    def mlp2_part(k, js):
        lhs = jnp.concatenate([_ld(a2, k, j) for j in js], axis=1)
        rhs = jnp.concatenate(
            [jnp.concatenate([ld_big(tile(49 + k, j) + 8 * n, 8) for j in js], axis=0) for n in range(2)],
            axis=1)
        return _dot(lhs, rhs)

    def merge(ms):
        c = _s_out(ms)
        return jnp.concatenate([jnp.concatenate(c[:2], axis=1), jnp.concatenate(c[2:], axis=1)], axis=0)

    unscale = 0.5 / GELU_S

    def finish(slot):
        ms = [mlp2_part(42 + k, range(NF)) for k in range(7)]
        obuf[slot, 0:HT, 0:D // 2] = (c11[...] + merge(ms) * unscale).astype(bf16)
        return [m[r:r + 16] for m in ms for r in range(0, QT, 16)]

    def phase2(b, carry):
        at = _Attn(flag[0], (sb0, sb1), (pb0, pb1))
        r0 = pl.multiple_of(b * T, T)

        def scores(u):
            return at.scores(u, qb_[pl.ds(r0 + u * HT, HT)], _ld(kb, _rows(r0 + u * HT, HT + W)),
                            b == 0, (W - u * HT) // 32)

        def values(u, pr):
            return at.values(pr([]), [_ld(vb, 2 * b + u + j) for j in range(3)])

        def o_blk(r, g):
            return ob[g, pl.ds(r0 + r * HT, HT)]

        def wo_op(i):
            if i == 1:
                return wo[0:D // 2, 0:D // 2]
            if i == 4:
                return wo[D // 2:D, D // 2:D]
            return jnp.concatenate([ld_big(otile((0, 2, 3, 5, 6).index(i), c), 32) for c in range(4)], axis=1)

        a11 = jnp.concatenate([o_blk(0, g) for g in range(4)], axis=1)
        a21 = jnp.concatenate([o_blk(1, g) for g in range(4)], axis=1)
        p0 = scores(0)
        m3 = _dot(a11, wo_op(2))
        o0 = values(0, p0)
        p1 = scores(1)
        m6 = _dot((a21.astype(f32) - a11.astype(f32)).astype(bf16), wo_op(5))
        o1 = values(1, p1)
        a12 = jnp.concatenate([o_blk(0, g).astype(f32) for g in range(4, NG - 1)] + [o0], axis=1)
        a22 = jnp.concatenate([o_blk(1, g).astype(f32) for g in range(4, NG - 1)] + [o1], axis=1)
        ops = _s_lhs(a11.astype(f32), a12, a21.astype(f32), a22)
        m = {2: m3, 5: m6}
        for i in (4, 1, 0, 3, 6):
            m[i] = _dot(ops[i].astype(bf16), wo_op(i))
        c = _s_out(m)
        h = xv[b].astype(f32) + jnp.concatenate(
            [jnp.concatenate(c[:2], axis=1), jnp.concatenate(c[2:], axis=1)], axis=0)

        ticks = [m[6][r:r + 16] for r in range(0, HT, 16)] + finish(b)
        y = _layernorm_chunks([h[QT * r + 16 * k:QT * r + 16 * k + 16] for k in range(4) for r in range(4)],
                              True, flag[0] > 0, OPT["lnlag"], OPT["lngate"], GELU_S, ticks[OPT["lt0"]:OPT["lt1"]])
        for k in range(4):
            for c in range(2):
                blk = [[y[4 * k + r][:, 256 * q + LG * c:256 * q + LG * (c + 1)]
                        for q in range(4)] for r in range(4)]
                for i, v in enumerate(_two_level(_s_lhs, blk)):
                    a1[i, c, 16 * k:16 * k + 16] = v.astype(bf16)

        z1 = flag[1] if OPT['z1'] else 0
        def act_steps(j, ms):
            inner, act = {}, {}

            def get_inner(k):
                if k not in inner:
                    inner[k] = [_s_out([m[16 * k:16 * k + 16] for m in ms[7 * i:7 * i + 7]]) for i in range(7)]
                return inner[k]

            def gelu_step(k, q):
                kv = GELU_A / GELU_S
                if newest:
                    kv = jnp.concatenate([jnp.where(flag[0] > 0, kv, newest[-1][0:8, 0:LG])] * 2, axis=0)
                for p, v in enumerate(_s_out([get_inner(k)[i][q] for i in range(7)])):
                    act[k, 2 * (p // 2) + q // 2, 2 * (p % 2) + q % 2] = _gelu_scaled(v, kv)

            def sum_step(k, o):
                ops = _two_level(_s_lhs, [[act[k, r, c] for c in range(4)] for r in range(4)])
                for i in range(7 * o, 7 * o + 7):
                    a2[i, j, 16 * k:16 * k + 16] = ops[i].astype(bf16)

            return [functools.partial(f, k, n) for k in range(4)
                    for f, cnt in ((gelu_step, 4), (sum_step, 7)) for n in range(cnt)]

        steps = []
        newest = []
        for j in range(NF):
            between = spread(steps, len(steps), OPT["actspan"])
            ms = []
            for i in range(49):
                ms.append(_dot(jnp.concatenate([_ld(a1, i + z1, c) for c in range(2)], axis=1),
                               ld_big(tile(i, j), 16)))
                if steps and i >= OPT['actfrom']:
                    newest.append(ms[-1])
                    between()
            for cc, i in enumerate((7 * 3 + 3, 7 * 3 + 2, 7 * 2 + 3, 7 * 2 + 2)):
                ms[i] = ms[i] + jnp.concatenate(
                    [bias[:, j * FC + cc * LG:j * FC + (cc + 1) * LG]] * (QT // 8), axis=0)
            steps = act_steps(j, ms)
        newest.clear()
        early = []
        between = spread(steps, len(steps), max(1, OPT["early"] - OPT["earlypad"]))
        for i in range(OPT["early"]):
            early.append(mlp2_part(i, range(4)))
            if steps:
                newest.append(early[-1])
                between()
        for f in steps:
            f()
        ms = [early[i] + mlp2_part(i, range(4, NF)) if i < len(early) else mlp2_part(i, range(NF))
              for i in range(42)]
        res = h + jnp.concatenate([bias[:, F:F + D]] * (T // 8), axis=0)
        m = [merge(ms[7 * i:7 * i + 7]) for i in range(6)]
        c11[...] = res[:HT, :D // 2] + (m[0] + m[3] - m[4]) * unscale
        obuf[b + 1, 0:HT, D // 2:D] = (res[:HT, D // 2:] + (m[2] + m[4]) * unscale).astype(bf16)
        obuf[b + 1, HT:T, 0:D // 2] = (res[HT:, :D // 2] + (m[1] + m[3]) * unscale).astype(bf16)
        obuf[b + 1, HT:T, D // 2:D] = (res[HT:, D // 2:] + (m[0] - m[1] + m[2] + m[5]) * unscale).astype(bf16)

        @pl.when(b > 0)
        def _():
            o_copy(b - 1).start()
        return carry

    lax.fori_loop(0, NB, phase2, None)
    finish(NB)
    o_copy(NB - 1).start()
    for i in range(NB):
        o_copy(i).wait()


@jax.jit
def pallas_sequential_preLN__sliding_block__mixer_channel_mlp__prompt_kernel(A_x, A_wqkv, A_wo, B_x, B_w1, B_b1, B_w2, B_b2):
    del B_x
    _, S, D = A_x.shape
    F = B_w1.shape[1]
    NB = S // T
    NG = D // LG
    NF = F // (4 * LG)
    hbm = pl.BlockSpec(memory_space=pl.ANY)
    vmem = pl.BlockSpec(memory_space=pltpu.VMEM)
    return pl.pallas_call(
        functools.partial(_kernel, S=S, D=D, F=F),
        out_shape=jax.ShapeDtypeStruct(A_x.shape, A_x.dtype),
        in_specs=[hbm, hbm, hbm, hbm, vmem, hbm, vmem],
        out_specs=hbm,
        scratch_shapes=[
            pltpu.VMEM((NB, T, D), bf16),
            pltpu.VMEM((NG, 3, D, LG), bf16),
            pltpu.VMEM((5, D // 2, LG), bf16),
            pltpu.VMEM((D, D), bf16),
            pltpu.VMEM((NF + 1, D, 4 * LG), bf16),
            pltpu.VMEM((NF + 1, 4 * LG, D), bf16),
            pltpu.VMEM((16 * 98 * NF + 8 * 36 * NB + 32 * 20, 16, LG), bf16),
            pltpu.VMEM((S, LG), bf16),
            pltpu.VMEM((W + S, LG), bf16),
            pltpu.VMEM(((W + S) // LG, LG, LG), bf16),
            pltpu.VMEM((NG - 1, S, LG), bf16),
            pltpu.VMEM((49, 2, T // 4, LG), bf16),
            pltpu.VMEM((49, NF, T // 4, LG), bf16),
            pltpu.VMEM((T // 2, D // 2), f32),
            pltpu.VMEM((8, F + D), f32),
            pltpu.VMEM((NB + 1, T, D), bf16),
            pltpu.VMEM((4, 8, 32, LG), f32),
            pltpu.VMEM((4, 8, 32, LG), f32),
            pltpu.VMEM((4, 384, LG), bf16),
            pltpu.VMEM((4, 384, LG), bf16),
            pltpu.VMEM((7, T // 2, LG), f32),
            pltpu.SMEM((8,), jnp.int32),
            pltpu.SemaphoreType.DMA((NB,)),
            pltpu.SemaphoreType.DMA((3, NG)),
            pltpu.SemaphoreType.DMA((NB,)),
        ],
        compiler_params=pltpu.CompilerParams(vmem_limit_bytes=124 * 2**20, flags=OPT["flags"] or None),
        name="fused_block",
    )(A_x, A_wqkv, A_wo, B_w1, B_b1, B_w2, B_b2)
```

```python
import functools
import math

import jax
import jax.numpy as jnp
from jax import lax
from jax.experimental import pallas as pl
from jax.experimental.pallas import tpu as pltpu

H = 32
W = 256
EPS = 1e-5
T = 256
HT = T // 2
QT = T // 4
LG = 128
MASKED = -1e30

GELU_A = math.sqrt(2.0 / math.pi)
GELU_S = (GELU_A * 0.044715) ** (1.0 / 3.0)

SCHEDULE = {
    "block": "s0 k012 q0:12 v0 s1 k345 k6:6 q1:12 v1 f",
    "block0": "s0 k012 k3:2 q0:14 v0 s1 k456 q1:12 w v1 f",
    "block1": "s0 k01 k2:4 q0:12 v0 s1 k345 k6:8 q1:8 v1 f",
    "block2": "s0 k012 q0:12 v0 s1 k345 k6:2 q1:12 v1 f",
    "block6": "s0 k012 q0:16 v0 s1 k3456 q1:8 v1 f",
    "block7": "s0 k01234 k5:2 q0:12 k6 v0 v1 f q1:0",
    "weight_steps": ((1, 5), (3,), (6,), (2, 4), (0,)),
    "projection": "d1 s1 m2 s0 m5 v1 d1 v0 m1 m0 t m346 d5",
    "projection_inner": (2, 0, 1, 4, 5, 6, 3),
    "norm_pace": (4, 6, 9, 12, 15, 17, 20, 23, 26, 27, 28, 30, 31, 32, 33, 35),
    "w1_first": (1, 5, 0, 2, 6, 3, 4),
    "w1_outer": (3, 1, 2, 6, 0, 4, 5),
    "gelu_span": 30,
    "w2_outer": (0, 3, 2, 1, 5, 4),
    "w2_inner": (0, 2, 3, 4, 1, 5, 6),
    "w2_split": 15,
}

f32 = jnp.float32
bf16 = jnp.bfloat16


def _cat(axis, parts):
    return jnp.concatenate(list(parts), axis=axis)


def _dot(a, b):
    return jnp.dot(a, b, preferred_element_type=f32)


def _after(always, value, other):
    return jnp.where(always, value, other)


def _tiles(ref, *idx):
    words = ref.bitcast(jnp.uint32)[idx]
    return pltpu.bitcast(words.reshape(-1, LG), bf16)


def _spread(steps, n, slots):
    calls = [0]

    def run():
        calls[0] += 1
        for _ in range(n * min(calls[0], slots) // slots - n * min(calls[0] - 1, slots) // slots):
            steps.pop(0)()
    return run if n else None


def _strassen_lhs(a11, a12, a21, a22):
    return [a11 + a22, a21 + a22, a11, a22, a11 + a12, a21 - a11, a12 - a22]


def _strassen_rhs(b11, b12, b21, b22):
    return [b11 + b22, b11, b12 - b22, b21 - b11, b22, b11 + b12, b21 + b22]


def _strassen_out(m):
    return [m[0] + m[3] - m[4] + m[6], m[2] + m[4], m[1] + m[3], m[0] - m[1] + m[2] + m[5]]


def _strassen_merge(m):
    c = _strassen_out(m)
    return _cat(0, [_cat(1, c[:2]), _cat(1, c[2:])])


def _two_levels(rule, blk):
    outer = [rule(*[blk[2 * r + i][2 * c + j] for r in range(2) for c in range(2)])
             for i in range(2) for j in range(2)]
    return [v for k in range(7) for v in rule(*[outer[q][k] for q in range(4)])]


def _layernorm(v, wait=None, twice=False, scale=1.0):
    mean = jnp.mean(v, axis=-1, keepdims=True)
    if wait is not None:
        mean = wait(mean)
    c = v - mean
    rs = lax.rsqrt(jnp.mean(c * c, axis=-1, keepdims=True) + EPS)
    if twice:
        c = c - jnp.mean(c, axis=-1, keepdims=True)
        var = jnp.mean(c * c, axis=-1, keepdims=True)
        rs = rs * lax.rsqrt(rs * rs * var + EPS)
    if scale != 1.0:
        rs = rs * scale
    return c * rs, rs


def _xor_shuffle(blocks, bit0, bit1):
    def select(mask, a, b):
        if a is None and b is None:
            return None
        return jnp.where(mask, jnp.zeros_like(b) if a is None else a, jnp.zeros_like(a) if b is None else b)

    swapped = [select(bit0, blocks[j ^ 1], blocks[j]) for j in range(4)]
    return [select(bit1, swapped[j ^ 2], swapped[j]) for j in range(4)]


class _Attention:
    def __init__(self, always, zero, score_refs):
        lane = lax.broadcasted_iota(jnp.int32, (32, LG), 1)
        self.bit0 = (lane & 32) != 0
        self.bit1 = (lane & 64) != 0
        self.head = [(lane >> 5) == h for h in range(4)]
        self.later = lax.broadcasted_iota(jnp.int32, (32, LG), 0) > (lane & 31)
        row = lax.broadcasted_iota(jnp.int32, (1, LG), 1)
        self.row_bits = ((row & 32) != 0, (row & 64) != 0)
        self.always, self.zero, self.score_refs = always, zero, score_refs

    def scores(self, slot, q, keys, first=None, before=0):
        skip = (W + 128 - keys.shape[0]) // 32
        ref = self.score_refs[slot]
        top, stored = [], set()
        for t in range(4):
            qt = q[32 * t:32 * t + 32].astype(f32)
            diag = _cat(0, [jnp.where(self.head[g ^ t], qt, 0.0) for g in range(4)]).astype(bf16)
            c0 = max(skip - t, 0)
            s = lax.dot_general(keys[32 * (t + c0 - skip):32 * (t + 9 - skip)], diag,
                                (((1,), (1,)), ((), ())), preferred_element_type=f32)
            s = {c: s[32 * (c - c0):32 * (c - c0 + 1)] for c in range(c0, 9)}
            if c0 > 0:
                s[0] = MASKED
            elif first is not None:
                s[0] = jnp.where(first, MASKED, s[0])
            s[0] = jnp.where(self.later, s[0], s.pop(8))
            old = 0 if first is None else before - t
            m = functools.reduce(jnp.maximum, [s[c] for c in range(max(1, old, c0), 8)] + [s[0]])
            if old > 1:
                m_old = functools.reduce(jnp.maximum, [s[c] for c in range(1, old)])
                m = jnp.maximum(m, jnp.where(first, MASKED, m_old))
            top.append(jnp.broadcast_to(jnp.max(m, axis=0, keepdims=True), (8, LG)))
            for c, v in s.items():
                ref[t, c] = v
                stored.add((t, c))
        return ref, skip, top, stored, first, before

    def values(self, scores, vt):
        ref, skip, top, stored, first, before = scores
        total, last, rows = [None] * 4, {}, []
        gate, fresh = None, []
        for r in range(12):
            for lo in (0, 16):
                blk = [None] * 4
                for t in range(4):
                    c = r - t
                    if c == 8:
                        blk[t] = last[t, lo]
                    if (t, c) not in stored:
                        continue
                    m = top[t] if gate is None else _after(self.always, top[t], gate)
                    if c > 0 and first is not None and r < before:
                        m = jnp.where(first, -MASKED, m)
                    p = jnp.exp2(ref[t + self.zero, c, lo:lo + 16] - _cat(0, [m, m]))
                    part = p[0:8] + p[8:16]
                    total[t] = part if total[t] is None else total[t] + part
                    fresh.append(t)
                    if c == 0:
                        last[t, lo] = jnp.where(self.later[lo:lo + 16], 0.0, p)
                        p = None if t < skip else jnp.where(self.later[lo:lo + 16], p, 0.0)
                    blk[t] = p
                if any(v is not None for v in blk):
                    rows.append(_xor_shuffle(blk, self.bit0[:16], self.bit1[:16]))
                if len(fresh) >= 3:
                    gate = functools.reduce(jnp.add, [total[t] for t in sorted(set(fresh))])
                    fresh = []
        inv = _xor_shuffle([1.0 / jnp.sum(v, axis=0, keepdims=True) for v in total], *self.row_bits)
        heads = [_dot(_cat(1, [v[32 * h:32 * h + 32] for v in vt]),
                      _cat(0, [row[h] for row in rows]).astype(bf16)) * inv[h] for h in range(4)]
        o = _cat(0, heads).T
        return _cat(0, _xor_shuffle([o[32 * g:32 * g + 32] for g in range(4)], self.bit0, self.bit1))


def _kernel(x_hbm, wqkv_hbm, wo_hbm, w1_hbm, b1_hbm, w2_hbm, b2_hbm, out_hbm,
            x, wqkv, wkv_sums, wo, w1, w2, ops, q, k, vt, attn, act, carried, b_raw, bias, out,
            scores0, scores1, kv_products, flags, x_sem, w_sem, out_sem):
    NB, _, D = x.shape
    NG = D // LG
    NF, FC, _ = w2.shape
    F = NF * FC
    HD = D // 2
    QD = D // 4
    SUMS = (0, 2, 3, 5, 6)
    q_scale = (D // H) ** -0.5 * math.log2(math.e)
    unscale = 0.5 / GELU_S

    def w_op(i, j):
        return 16 * (98 * j + i)

    def y_op(b, i, c):
        return w_op(0, NF) + 8 * (4 * (9 * b + i) + c)

    def wo_op(i, c):
        return y_op(NB, 0, 0) + 16 * (2 * i + c)

    def load_op(at, n):
        return _tiles(ops, pl.ds(at, n))

    def x_copy(b):
        return pltpu.make_async_copy(x_hbm.at[0, pl.ds(b * T, T)], x.at[b], x_sem.at[b])

    def out_copy(b):
        return pltpu.make_async_copy(out.at[b + 1], out_hbm.at[0, pl.ds(b * T, T)], out_sem.at[b])

    def qkv_copy(g, p):
        return pltpu.make_async_copy(wqkv_hbm.at[:, pl.ds((p + 1) % 3 * D + g * LG, LG)],
                                     wqkv.at[pl.ds((3 * g + p) * D, D)], w_sem.at[p // 2, g])

    def wo_copy(g):
        return pltpu.make_async_copy(wo_hbm.at[:, pl.ds(16 * g, 16)], wo.at[g], w_sem.at[2, g])

    def step_copies(g):
        return [qkv_copy(g + 1, p) for p in range(3)] + [
            pltpu.make_async_copy(w1_hbm.at[:, pl.ds(g * FC, FC)], w1.at[g], w_sem.at[2, g]),
            pltpu.make_async_copy(w2_hbm.at[pl.ds(g * FC, FC), :], w2.at[g], w_sem.at[2, g]), wo_copy(g)]

    def late_copies():
        return [wo_copy(NF)] + [pltpu.make_async_copy(src, dst, w_sem.at[2, NF]) for src, dst in (
            (b1_hbm, b_raw.at[pl.ds(0, F)]), (b2_hbm, b_raw.at[pl.ds(b_raw.shape[0] // 2, D)]))]

    x_copy(0).start()
    for p in range(3):
        qkv_copy(0, p).start()
    x_copy(1).start()

    k[0:W] = jnp.zeros((W, LG), bf16)
    vt[0:W // LG] = jnp.zeros((W // LG, LG, LG), bf16)
    act[42:49] = jnp.zeros((7,) + act.shape[1:], bf16)
    carried[...] = jnp.zeros_like(carried)
    flags[0] = 1
    flags[1] = 0

    def normalize_input(b, lag):
        ys, factors = [], []
        for lo in range(0, HT, 16):
            for r in range(2):
                wait = None
                if 0 < lag <= len(factors):
                    wait = functools.partial(_after, flags[0] > 0, other=factors[-lag])
                y, rs = _layernorm(x[b, r * HT + lo:r * HT + lo + 16].astype(f32), wait)
                ys.append(y)
                factors.append(rs)
        for n in range(HT // 16):
            for c in range(4):
                blk = [ys[2 * n + r][:, p * HD + c * LG:p * HD + (c + 1) * LG] for r in range(2) for p in range(2)]
                for i, v in enumerate(_strassen_lhs(*blk) + blk[1:3]):
                    ops[y_op(b, 0, 0) + (y_op(0, i, c) - y_op(0, 0, 0) + n)] = v.astype(bf16)

    def load_y(b, i, between):
        if between is None:
            return _cat(1, [load_op(y_op(b, i, c), 8) for c in range(4)])
        zero, rows = flags[1], []
        for n in range(HT // 16):
            between()
            rows.append(_cat(1, [load_op(zero + (y_op(b, i, c) + n), 1) for c in range(4)]))
        return _cat(0, rows)

    def load_wqkv(g, p, lo, n):
        start = 3 * HD * g + (p * D + lo) // 2
        return _tiles(wqkv, pl.ds(start if isinstance(start, int) else pl.multiple_of(start, 8), n // 2))

    def project_q(g, b, r, between=None):
        wq = load_wqkv(g, 2, 0, D)
        y = _cat(1, [load_y(b, i, between) for i in ((2, 7), (8, 3))[r]])
        q[pl.ds(b * T + r * HT, HT)] = (_dot(y, wq) * q_scale).astype(bf16)

    def prepare_kv(g):
        blk = [load_wqkv(g, p, r * HD, HD) for r in range(2) for p in range(2)]
        for lo in range(0, HD, 16):
            sums = _strassen_rhs(*[v[lo:lo + 16].astype(f32) for v in blk])
            for n, i in enumerate(SUMS):
                wkv_sums[n, lo:lo + 16] = sums[i].astype(bf16)

    def kv_product(g, b, i, between=None):
        if i in SUMS:
            rhs = _tiles(wkv_sums, SUMS.index(i))
        else:
            rhs = load_wqkv(g, i // 4, i // 4 * HD, HD)
        m = _dot(load_y(b, i, between), rhs)
        if i < 6:
            kv_products[i] = m
        return m

    def store_kv(b, m):
        c = _strassen_out([kv_products[i + flags[0] - 1] for i in range(6)] + [m[6]])
        for r in range(2):
            k[pl.ds(W + b * T + r * HT, HT)] = c[2 * r].astype(bf16)
            vt[2 + 2 * b + r] = c[2 * r + 1].T.astype(bf16)

    def store_operands(blk, outer, at):
        sums = _two_levels(_strassen_rhs, blk)
        for i in (7 * u + v for u in outer for v in range(7)):
            ops[at(i)] = sums[i].astype(bf16)

    def prepare_w1(j, n, outer):
        store_operands([[w1[j, pl.ds(QD * r + 16 * n, 16), c * LG:(c + 1) * LG].astype(f32)
                         for c in range(4)] for r in range(4)],
                       outer, lambda i: w_op(0, j) + (w_op(i, 0) + n))

    def prepare_w2(j, n, outer):
        col, row = divmod(n, 8)
        store_operands([[w2[j, pl.ds(LG * r + 16 * row, 16), QD * c + LG * col:QD * c + LG * (col + 1)].astype(f32)
                         for c in range(4)] for r in range(4)],
                       outer, lambda i: w_op(0, j) + (w_op(49 + i, 0) + n))

    def prepare_wo(j, n, outer):
        col, row = divmod(n, 2)
        store_operands([[wo[j, 2 * r + row, :, QD * c + LG * col:QD * c + LG * (col + 1)].astype(f32)
                         for c in range(4)] for r in range(4)],
                       outer, lambda i: j + (wo_op(i, col) + 8 * row))

    x_copy(0).wait()
    for b in (2, 3):
        x_copy(b).start()
    normalize_input(0, 0)
    for p in range(2):
        qkv_copy(0, p).wait()
    for b in range(4, NB):
        x_copy(b).start()
    prepare_kv(0)
    store_kv(0, [kv_product(0, 0, i) for i in range(7)])
    qkv_copy(0, 2).wait()
    x_copy(1).wait()
    for cp in step_copies(0):
        cp.start()
    for r in range(2):
        project_q(0, 0, r)
    normalize_input(1, 0)

    def phase0(b, carry):
        x_copy(b + 1).wait()
        store_kv(b, [kv_product(0, b, i) for i in range(7)])
        for r in range(2):
            project_q(0, b, r)
        normalize_input(b + 1, 2)
        return carry

    lax.fori_loop(1, NB - 1, phase0, None)
    for cp in step_copies(1) + step_copies(2):
        cp.start()

    def phase1(g, carry):
        for cp in step_copies(g):
            cp.wait()

        @pl.when(g == 1)
        def _():
            for cp in [cp for j in range(3, NF) for cp in step_copies(j)] + late_copies():
                cp.start()

        att = _Attention(flags[0] > 0, flags[0] - 1, (scores0, scores1))

        def scores(u):
            lo = max(u * HT, W)
            return att.scores(u % 2, q[u * HT:(u + 1) * HT],
                              _tiles(k, pl.ds(lo // 2, ((u + 1) * HT + W - lo) // 2)))

        steps = [functools.partial(prepare, g, n, outer)
                 for n in range(16) for prepare in (prepare_w1, prepare_w2) for outer in SCHEDULE["weight_steps"]]
        steps += [functools.partial(prepare_wo, g, n, outer) for n in range(4) for outer in SCHEDULE["weight_steps"]]
        orders = [[op.partition(":") for op in SCHEDULE.get("block%d" % b, SCHEDULE["block"]).split()]
                  for b in range(NB)]
        weight = sum(int(share or 0) for order in orders for _, _, share in order)
        count, used = len(steps), 0
        pending = {0: scores(0)}
        for b, order in enumerate(orders):
            gp, bp = (g, NB - 1) if b == 0 else (g + 1, b - 1)
            m = []
            for op, _, share in order:
                n = count * (used + int(share or 0)) // weight - count * used // weight
                used += int(share or 0)
                if op[0] == "s":
                    u = 2 * b + 1 + int(op[1])
                    pending[u] = scores(u)
                elif op[0] == "v":
                    u = 2 * b + int(op[1])
                    o = att.values(pending.pop(u), [_tiles(vt, j) for j in range(max(u, 2), u + 3)])
                    attn[g, u * HT:(u + 1) * HT] = o.astype(bf16)
                elif op[0] == "k":
                    between = _spread(steps, n, 8 * len(op[1:]))
                    m += [kv_product(gp, bp, int(i), between) for i in op[1:]]
                elif op[0] == "q":
                    project_q(gp, bp, int(op[1]), _spread(steps, n, 16))
                elif op[0] == "f":
                    store_kv(bp, m)
                else:
                    prepare_kv(g + 1)
        return carry

    lax.fori_loop(0, NG - 1, phase1, None)

    for cp in late_copies():
        cp.wait()
    b2_at = b_raw.shape[0] // 2
    bias[:, 0:F] = jnp.broadcast_to(b_raw[0:F].astype(f32).reshape(1, F) * GELU_S, (8, F))
    bias[:, F:F + D] = jnp.broadcast_to(b_raw[b2_at:b2_at + D].astype(f32).reshape(1, D), (8, D))
    steps = [functools.partial(prepare_wo, NF, n, outer) for n in range(4) for outer in SCHEDULE["weight_steps"]]
    between = _spread(steps, len(steps), 56)
    store_kv(NB - 1, [kv_product(NG - 1, NB - 1, i, between) for i in range(7)])
    for r in range(2):
        project_q(NG - 1, NB - 1, r)

    def w2_product(i, js=range(NF)):
        return _dot(_cat(1, [_tiles(act, i, j) for j in js]),
                    _cat(1, [_cat(0, [load_op(w_op(49 + i, j) + 8 * col, 8) for j in js]) for col in range(2)]))

    def finish(slot, products):
        out[slot, 0:HT, 0:HD] = (carried[...] + _strassen_merge(products) * unscale).astype(bf16)

    def phase2(b, carry):
        always = flags[0] > 0
        att = _Attention(always, flags[0] - 1, (scores0, scores1))
        row = pl.multiple_of(b * T, T)

        def heads(r, groups):
            return [attn[g, pl.ds(row + r * HT, HT)].astype(f32) for g in groups]

        pending, o, m, left_over, pace = {}, {}, {}, [], []
        for op in SCHEDULE["projection"].split():
            if op[0] == "s":
                u = int(op[1])
                keys = _tiles(k, pl.ds(pl.multiple_of((row + u * HT) // 2, 8), (HT + W) // 2))
                pending[u] = att.scores(u, q[pl.ds(row + u * HT, HT)], keys, b == 0, (W - u * HT) // 32)
            elif op[0] == "v":
                u = int(op[1])
                o[u] = att.values(pending[u], [_tiles(vt, 2 * b + u + j) for j in range(3)])
            elif op[0] == "d":
                for _ in range(int(op[1])):
                    left_over.append(w2_product(42 + len(left_over)))
                    pace += [left_over[-1][r:r + 16] for r in range(0, QT, 16)]
            elif op[0] == "t":
                pace = []
            else:
                for i in map(int, op[1:]):
                    left = [_cat(1, heads(r, range(4))) for r in range(2)]
                    right = [_cat(1, heads(r, range(4, NG - 1)) + [o[r]]) if r in o else 0.0 for r in range(2)]
                    a = _strassen_lhs(left[0], right[0], left[1], right[1])[i]
                    a = _strassen_lhs(a[:QT, :QD], a[:QT, QD:], a[QT:, :QD], a[QT:, QD:])
                    inner = [None] * 7
                    for n in SCHEDULE["projection_inner"]:
                        inner[n] = _dot(a[n].astype(bf16),
                                        _cat(1, [load_op(wo_op(7 * i + n, col), 16) for col in range(2)]))
                        pace.append(inner[n][0:16])
                    pace.append(inner[n][48:64])
                    m[i] = _strassen_merge(inner)
        finish(b, left_over)

        xs = [x[b, r * HT:(r + 1) * HT, c * HD:(c + 1) * HD].astype(f32) for r in range(2) for c in range(2)]
        h = _cat(0, [_cat(1, [xs[0] + m[0] + m[3] - m[4] + m[6], xs[1] + m[2] + m[4]]),
                     _cat(1, [xs[2] + m[1] + m[3], xs[3] + m[2] + m[5] - m[1] + m[0]])])
        y = {}
        for n, r in [(n, r) for half in ((2, 3), (0, 1)) for n in range(4) for r in half]:
            wait = functools.partial(_after, always, other=pace[SCHEDULE["norm_pace"][len(y)]][:, 0:1])
            y[n, r], _ = _layernorm(h[QT * r + 16 * n:QT * r + 16 * n + 16], wait, twice=True, scale=GELU_S)
        lhs = [[_two_levels(_strassen_lhs, [[y[n, r][:, QD * c + LG * col:QD * c + LG * (col + 1)]
                                             for c in range(4)] for r in range(4)])
                for col in range(2)] for n in range(4)]
        lhs = [_cat(0, [_cat(1, [lhs[n][col][i] for col in range(2)]) for n in range(4)]).astype(bf16)
               for i in range(49)]

        newest = []

        def activation_steps(j, products):
            inner, gelu = {}, {}

            def activate(n, s):
                slope = GELU_A / GELU_S
                if newest:
                    slope = _cat(0, [_after(always, slope, newest[-1][0:8, 0:LG])] * 2)
                if n not in inner:
                    inner[n] = [_strassen_out([v[16 * n:16 * n + 16] for v in products[i:i + 7]])
                                for i in range(0, 49, 7)]
                for p, u in enumerate(_strassen_out([v[s] for v in inner[n]])):
                    gelu[n, 2 * (p // 2) + s // 2, 2 * (p % 2) + s % 2] = u + u * jnp.tanh(u * (slope + u * u))

            def store(n):
                blk = [[gelu[n, r, c] for c in range(4)] for r in range(4)]
                for i, v in enumerate(_two_levels(_strassen_lhs, blk)):
                    act[i, j, 16 * n:16 * n + 16] = v.astype(bf16)

            return [step for n in range(4) for step in (
                [functools.partial(activate, n, s) for s in range(4)]
                + [functools.partial(store, n)] + [lambda: None] * 6)]

        steps = []
        for j in range(NF):
            between = _spread(steps, len(steps), SCHEDULE["gelu_span"])
            products = {}
            for i in (7 * u + v for u in SCHEDULE["w1_outer" if j else "w1_first"] for v in range(7)):
                products[i] = _dot(lhs[i], load_op(w_op(i, j), 16))
                if steps:
                    newest.append(products[i])
                    between()
            for c, i in enumerate((7 * 3 + 3, 7 * 3 + 2, 7 * 2 + 3, 7 * 2 + 2)):
                products[i] = products[i] + _cat(0, [bias[:, j * FC + c * LG:j * FC + (c + 1) * LG]] * (QT // 8))
            steps = activation_steps(j, [products[i] for i in range(49)])
        between = _spread(steps, len(steps), SCHEDULE["w2_split"] - 1)
        order = [7 * u + v for u in SCHEDULE["w2_outer"] for v in SCHEDULE["w2_inner"]]
        products = {}
        for i in order[:SCHEDULE["w2_split"]]:
            products[i] = w2_product(i, range(4))
            newest.append(products[i])
            between()
        for i in order:
            products[i] = products[i] + w2_product(i, range(4, NF)) if i in products else w2_product(i)
        res = h + _cat(0, [bias[:, F:F + D]] * (T // 8))
        m = [_strassen_merge([products[i + v] for v in range(7)]) for i in range(0, 42, 7)]
        carried[...] = res[:HT, :HD] + (m[0] + m[3] - m[4]) * unscale
        out[b + 1, 0:HT, HD:D] = (res[:HT, HD:] + (m[2] + m[4]) * unscale).astype(bf16)
        out[b + 1, HT:T, 0:HD] = (res[HT:, :HD] + (m[1] + m[3]) * unscale).astype(bf16)
        out[b + 1, HT:T, HD:D] = (res[HT:, HD:] + (m[0] - m[1] + m[2] + m[5]) * unscale).astype(bf16)

        @pl.when(b > 0)
        def _():
            out_copy(b - 1).start()
        return carry

    lax.fori_loop(0, NB, phase2, None)

    tail = [pltpu.make_async_copy(out.at[NB, pl.ds(r, HT), pl.ds(c, n)],
                                  out_hbm.at[0, pl.ds((NB - 1) * T + r, HT), pl.ds(c, n)], out_sem.at[NB - 1 + i])
            for i, (r, c, n) in enumerate(((HT, 0, D), (0, HD, HD), (0, 0, HD)))]
    tail[0].start()
    tail[1].start()
    finish(NB, [w2_product(i) for i in range(42, 49)])
    tail[2].start()
    for cp in [out_copy(b) for b in range(NB - 1)] + tail:
        cp.wait()


@jax.jit
def pallas_sequential_preLN__sliding_block__mixer_channel_mlp__prompt_kernel(
    A_x: jax.Array,
    A_wqkv: jax.Array,
    A_wo: jax.Array,
    B_x: jax.Array,
    B_w1: jax.Array,
    B_b1: jax.Array,
    B_w2: jax.Array,
    B_b2: jax.Array,
):
    del B_x
    _, S, D = A_x.shape
    F = B_w1.shape[1]
    NB, NG, NF = S // T, D // LG, F // (4 * LG)
    assert A_x.shape[0] == 1 and S == NB * T and D == 32 * H and F == 4 * LG * (NG - 1)
    hbm = pl.BlockSpec(memory_space=pl.ANY)
    return pl.pallas_call(
        _kernel,
        out_shape=jax.ShapeDtypeStruct(A_x.shape, A_x.dtype),
        in_specs=[hbm] * 7,
        out_specs=hbm,
        scratch_shapes=[
            pltpu.VMEM((NB, T, D), bf16),
            pltpu.VMEM((NG * 3 * D, LG), bf16),
            pltpu.VMEM((5, D // 2, LG), bf16),
            pltpu.VMEM((NG, 8, 16, D), bf16),
            pltpu.VMEM((NF, D, 4 * LG), bf16),
            pltpu.VMEM((NF, 4 * LG, D), bf16),
            pltpu.VMEM((16 * 98 * NF + 8 * 36 * NB + 32 * 49, 16, LG), bf16),
            pltpu.VMEM((S, LG), bf16),
            pltpu.VMEM((W + S, LG), bf16),
            pltpu.VMEM(((W + S) // LG, LG, LG), bf16),
            pltpu.VMEM((NG - 1, S, LG), bf16),
            pltpu.VMEM((49, NF, QT, LG), bf16),
            pltpu.VMEM((HT, D // 2), f32),
            pltpu.VMEM((8192,), bf16),
            pltpu.VMEM((8, F + D), f32),
            pltpu.VMEM((NB + 1, T, D), bf16),
            pltpu.VMEM((4, 8, 32, LG), f32),
            pltpu.VMEM((4, 8, 32, LG), f32),
            pltpu.VMEM((6, HT, LG), f32),
            pltpu.SMEM((2,), jnp.int32),
            pltpu.SemaphoreType.DMA((NB,)),
            pltpu.SemaphoreType.DMA((3, NG)),
            pltpu.SemaphoreType.DMA((NB + 2,)),
        ],
        compiler_params=pltpu.CompilerParams(vmem_limit_bytes=120 * 2**20),
        name="fused_block",
    )(A_x, A_wqkv, A_wo.reshape(8, D // 8, D), B_w1, B_b1, B_w2, B_b2)
```
